```python
import jax
import jax.numpy as jnp

def _softmax(x, axis=-1):
    return jax.nn.softmax(x, axis=axis)
def _gelu(x):
    return jax.nn.gelu(x, approximate=True)
def _silu(x):
    return jax.nn.silu(x)
def _sigmoid(x):
    return jax.nn.sigmoid(x)
def _layernorm(x, axis=-1, eps=1e-5):
    m = jnp.mean(x, axis=axis, keepdims=True)
    v = jnp.var(x, axis=axis, keepdims=True)
    return (x - m) / jnp.sqrt(v + eps)
def _scatter_add(tgt, idx, src, axis=0):
    return tgt.at[idx].add(src)
def _segment_sum(src, seg, n):
    return jax.ops.segment_sum(src, seg, n)
class _Rng:
    def __init__(self, key):
        self._k = key
    def _next(self):
        self._k, sub = jax.random.split(self._k)
        return sub
    def normal(self, shape):
        return jax.random.normal(self._next(), shape, dtype=jnp.bfloat16)
    def randint(self, lo, hi, shape):
        return jax.random.randint(self._next(), shape, lo, hi, dtype=jnp.int32)
    def uniform(self, shape, lo=0.0, hi=1.0):
        return jax.random.uniform(self._next(), shape, jnp.bfloat16, lo, hi)
    def permutation(self, n):
        return jax.random.permutation(self._next(), n)


kernel_name = 'standalone__standard_2d_1d_3d_conv__vision'

def setup_inputs():
    _rng = _Rng(jax.random.key(int.from_bytes(__import__("os").urandom(4), "little")))
    _w = (lambda a: (lambda t: t.astype(jnp.bfloat16) if jnp.issubdtype(t.dtype, jnp.floating) else t)(jnp.asarray(a)))
    H = W = 384
    C = 384
    K = 1
    return {
        "x": _w((lambda *s: _rng.normal(s) * 0.05)(1, H, W, C)),
        "w": _w((lambda *s: _rng.normal(s) * 0.05)(K, K, C, C)),
        "b": _w((lambda *s: _rng.normal(s) * 0.05)(C)),
    }

def reference(x, w, b):
    B, H, W, Cin = x.shape
    K = w.shape[0]
    pl = (K - 1) // 2
    pr = K // 2
    xp = jnp.pad(x, ((0, 0), (pl, pr), (pl, pr), (0, 0)))
    out = sum(
        jnp.einsum('bhwc,cd->bhwd', xp[:, i:i+H, j:j+W, :], w[i, j])
        for i in range(K) for j in range(K)
    )
    return out + b[None, None, None, :]
```

```python
import jax
import jax.numpy as jnp
from jax import lax
import jax.experimental.pallas as pl
import jax.experimental.pallas.tpu as pltpu

_CH = 1024
_RD = 128
_AHEAD = 6
_P = 32
_S = 1024
_A = 16
_W_AHEAD = 64


def _conv1x1_kernel(x_hbm, w_ref, b_ref, o_hbm, buf, rsems, wsem):
    m, c = buf.shape
    n = m // _CH
    group_rows = _A * _S
    per_group = _S // _P
    n_writes = (m // group_rows) * per_group
    steps_per_group = group_rows // _CH
    switch = n // 2
    n_read_steps = (n - _AHEAD) // 2
    writes_per_step = 3 * _CH // (2 * _A * _P)

    bias = b_ref[...].astype(jnp.float32).reshape(1, c)
    o_view = o_hbm.reshape(m // _S, per_group, _P, c)
    buf_view = buf.reshape(m // _S, per_group, _P, c)

    def start_read(i):
        for k in range(_CH // _RD):
            r0 = pl.multiple_of(i * _CH + k * _RD, _RD)
            pltpu.make_async_copy(
                x_hbm.at[pl.ds(r0, _RD)], buf.at[pl.ds(r0, _RD)], rsems.at[i]
            ).start(priority=k % 2)

    def wait_read(i):
        r0 = pl.multiple_of(i * _CH, _CH)
        pltpu.make_async_copy(
            x_hbm.at[pl.ds(r0, _CH)], buf.at[pl.ds(r0, _CH)], rsems.at[i]
        ).wait()

    def start_write(u):
        g, j = u // per_group, u % per_group
        pltpu.make_async_copy(
            buf_view.at[pl.ds(g * _A, _A), j], o_view.at[pl.ds(g * _A, _A), j], wsem
        ).start()

    def writes_issued(k):
        return jnp.minimum(
            _W_AHEAD + k * writes_per_step,
            ((switch + k) // steps_per_group) * per_group,
        )

    for i in range(_AHEAD):
        start_read(i)

    def step(i, carry):
        @pl.when(i < n_read_steps)
        def _():
            start_read(2 * i + _AHEAD)
            start_read(2 * i + _AHEAD + 1)

        @pl.when(i < switch)
        def _():
            wait_read(i)

        @pl.when(i == switch)
        def _():
            def wait_body(j, carry):
                wait_read(j)
                return carry

            lax.fori_loop(switch, n - 1, wait_body, 0)
            for u in range(_W_AHEAD):
                start_write(u)
            wait_read(n - 1)

        blk = buf.at[pl.ds(pl.multiple_of(i * _CH, _CH), _CH)]
        acc = jnp.dot(blk[...], w_ref[...], preferred_element_type=jnp.float32)
        blk[...] = (acc + bias).astype(blk.dtype)

        @pl.when(i >= switch)
        def _():
            def write_body(u, carry):
                start_write(u)
                return carry

            hi = jnp.where(i == n - 1, n_writes, writes_issued(i - switch + 1))
            lax.fori_loop(writes_issued(i - switch), hi, write_body, 0)

        return carry

    lax.fori_loop(0, n, step, 0)
    pltpu.make_async_copy(buf, o_hbm, wsem).wait()


@jax.jit
def pallas_standalone__standard_2d_1d_3d_conv__vision_kernel(
    x: jax.Array,
    w: jax.Array,
    b: jax.Array,
):
    batch, height, width, cin = x.shape
    kh, kw, _, cout = w.shape
    assert (kh, kw) == (1, 1) and cin == cout
    m = batch * height * width
    out = pl.pallas_call(
        _conv1x1_kernel,
        in_specs=[
            pl.BlockSpec(memory_space=pltpu.HBM),
            pl.BlockSpec(memory_space=pltpu.VMEM),
            pl.BlockSpec(memory_space=pltpu.VMEM),
        ],
        out_specs=pl.BlockSpec(memory_space=pltpu.HBM),
        out_shape=jax.ShapeDtypeStruct((m, cout), x.dtype),
        scratch_shapes=[
            pltpu.VMEM((m, cin), x.dtype),
            pltpu.SemaphoreType.DMA((m // _CH,)),
            pltpu.SemaphoreType.DMA(()),
        ],
        compiler_params=pltpu.CompilerParams(vmem_limit_bytes=120 * 2**20),
    )(x.reshape(m, cin), w.reshape(cin, cout), b)
    return out.reshape(batch, height, width, cout)
```

```python
import jax
import jax.numpy as jnp
from jax import lax
import jax.experimental.pallas as pl
import jax.experimental.pallas.tpu as pltpu

_BLOCK = 4096
_STARTS = (0, 1368, 2728)
_BODY = 1344
_REST = tuple(
    end - start - _BODY for start, end in zip(_STARTS, _STARTS[1:] + (_BLOCK,))
)

_READ_ROWS = 24
_WRITE_ROWS = 48
_CHUNK1 = 96
_CHUNK2 = 192
_AHEAD = 2
_RING = 4
_TAIL = 3
_WRITE_STEPS = 4
_LEAD = 4
_REST_UNITS = 9


def _conv1x1_kernel(x_hbm, w_hbm, b_hbm, o_hbm, buf, w_ref, b_ref, ring, bulk):
    c = buf.shape[-1]
    groups = buf.shape[0] // 4
    steps1, steps2 = _BODY // _CHUNK1, _BODY // _CHUNK2
    n1, n2 = groups * steps1, groups * steps2
    n_write_steps = 2 * groups * _WRITE_STEPS
    sweeps = _CHUNK1 // _READ_ROWS
    switch = n1 - _AHEAD + 1
    param_sem = ring.at[_RING - 1]
    tail_sem = ring.at[n1 % _RING]

    def copy(src, dst, unit, row, rows, sem, thread):
        idx = (pl.ds(2 * unit, 2), pl.ds(row, rows))
        pltpu.make_async_copy(src.at[idx], dst.at[idx], sem).start(priority=thread)

    def wait(blocks, rows, sem):
        size = buf.at[pl.ds(0, blocks), pl.ds(0, rows)]
        pltpu.make_async_copy(size, size, sem).wait()

    def read_step(i, last=False):
        g = i // steps1 if last else lax.div(i, steps1)
        j = i - g * steps1
        base = j * _CHUNK1 if last else pl.multiple_of(j * _CHUNK1, 8)
        for s in range(sweeps):
            in_tail = last and s >= sweeps - _TAIL
            for start in _STARTS:
                row = base + start + s * _READ_ROWS
                copy(x_hbm, buf, 2 * g, row, _READ_ROWS, ring.at[i & (_RING - 1)], 0)
                copy(x_hbm, buf, 2 * g + 1, row, _READ_ROWS,
                     tail_sem if in_tail else bulk, 1)

        def read_rest():
            for start, rows in zip(_STARTS, _REST):
                for h in range(2):
                    copy(x_hbm, buf, 2 * g + h, start + _BODY, rows,
                         tail_sem if last else bulk, h)

        if last:
            read_rest()
        else:
            pl.when(j == steps1 - 1)(read_rest)

    def write_steps(lo, hi):
        rows_per_step = _BODY // _WRITE_STEPS

        def body(m, carry):
            v = lax.div(m, _WRITE_STEPS)
            r = m - v * _WRITE_STEPS
            unit = jnp.where(v < groups, 2 * v, 2 * (v - groups) + 1)
            base = pl.multiple_of(r * rows_per_step, 8)
            for s in range(rows_per_step // _WRITE_ROWS):
                for start in _STARTS:
                    copy(buf, o_hbm, unit, base + start + s * _WRITE_ROWS,
                         _WRITE_ROWS, bulk, 0)

            @pl.when(r == _WRITE_STEPS - 1)
            def _():
                for start, rows in zip(_STARTS, _REST):
                    copy(buf, o_hbm, unit, start + _BODY, rows, bulk, 0)

            return carry

        lax.fori_loop(lo, hi, body, 0)

    def matmul(view, starts, sizes):
        blocks = view.shape[0]
        lhs = jnp.concatenate([
            view[:, pl.ds(start, rows), :].reshape(blocks * rows, c)
            for start, rows in zip(starts, sizes)
        ])
        acc = jnp.dot(lhs, w_ref[...], preferred_element_type=jnp.float32)
        out = (acc + bias).astype(buf.dtype)
        row = 0
        for start, rows in zip(starts, sizes):
            piece = out[row:row + blocks * rows]
            view[:, pl.ds(start, rows), :] = piece.reshape(blocks, rows, c)
            row += blocks * rows

    def compute(unit, j, chunk):
        base = pl.multiple_of(j * chunk, 8)
        view = buf.at[pl.ds(2 * unit, 2), pl.ds(base, _STARTS[-1] + chunk)]
        matmul(view, _STARTS, (chunk,) * len(_STARTS))

    w_copy = pltpu.make_async_copy(w_hbm, w_ref, param_sem)
    b_copy = pltpu.make_async_copy(b_hbm, b_ref, param_sem)

    def prologue(i, carry):
        read_step(i)

        @pl.when(i == 0)
        def _():
            w_copy.start()
            b_copy.start()

        return carry

    lax.fori_loop(0, _AHEAD, prologue, 0)
    w_copy.wait()
    b_copy.wait()
    bias = b_ref[...].astype(jnp.float32).reshape(1, c)

    def phase1(i, carry):
        @pl.when(i + _AHEAD < n1 - 1)
        def _():
            read_step(i + _AHEAD)

        @pl.when(i + _AHEAD == n1 - 1)
        def _():
            read_step(n1 - 1, last=True)

        @pl.when(i < switch)
        def _():
            wait(2, len(_STARTS) * _CHUNK1, ring.at[i & (_RING - 1)])

        @pl.when(i == switch)
        def _():
            for t in range(switch, n1):
                wait(2, len(_STARTS) * _CHUNK1, ring.at[t % _RING])
            wait(4 * (groups - 1), sum(_REST), bulk)
            wait(2 * (groups - 1), len(_STARTS) * _BODY, bulk)
            wait(2, len(_STARTS) * (_BODY - _TAIL * _READ_ROWS), bulk)
            write_steps(0, _WRITE_STEPS - 1)
            wait(2, len(_STARTS) * _TAIL * _READ_ROWS + 2 * sum(_REST), tail_sem)

        g = lax.div(i, steps1)
        compute(2 * g, i - g * steps1, _CHUNK1)
        return carry

    lax.fori_loop(0, n1, phase1, 0)

    def rest(u, carry):
        view = buf.at[pl.ds(u * 2 * _REST_UNITS, 2 * _REST_UNITS)]
        matmul(view, [start + _BODY for start in _STARTS], _REST)
        return carry

    lax.fori_loop(0, 2 * groups // _REST_UNITS, rest, 0)
    write_steps(_WRITE_STEPS - 1, _LEAD)

    for k in range(1, n2 + 1):
        g, j = divmod(k, steps2)
        assert _LEAD + k <= (groups + g) * _WRITE_STEPS + j * _WRITE_STEPS // steps2

    def phase2(k, carry):
        g = lax.div(k, steps2)
        compute(2 * g + 1, k - g * steps2, _CHUNK2)
        write_steps(_LEAD + k, jnp.where(k == n2 - 1, n_write_steps, _LEAD + k + 1))
        return carry

    lax.fori_loop(0, n2, phase2, 0)
    pltpu.make_async_copy(buf, o_hbm, bulk).wait()


@jax.jit
def pallas_standalone__standard_2d_1d_3d_conv__vision_kernel(
    x: jax.Array,
    w: jax.Array,
    b: jax.Array,
):
    batch, height, width, cin = x.shape
    kh, kw, _, cout = w.shape
    blocks = batch * height * width // _BLOCK
    assert (kh, kw) == (1, 1) and cin == cout
    assert blocks * _BLOCK == batch * height * width
    assert blocks % 4 == 0 and blocks % (2 * _REST_UNITS) == 0
    hbm = pl.BlockSpec(memory_space=pltpu.HBM)
    out = pl.pallas_call(
        _conv1x1_kernel,
        in_specs=[hbm, hbm, hbm],
        out_specs=hbm,
        out_shape=jax.ShapeDtypeStruct((blocks, _BLOCK, cout), x.dtype),
        scratch_shapes=[
            pltpu.VMEM((blocks, _BLOCK, cin), x.dtype),
            pltpu.VMEM((cin, cout), w.dtype),
            pltpu.VMEM((cout,), b.dtype),
            pltpu.SemaphoreType.DMA((_RING,)),
            pltpu.SemaphoreType.DMA(()),
        ],
        compiler_params=pltpu.CompilerParams(
            vmem_limit_bytes=120 * 2**20,
            disable_bounds_checks=True,
        ),
    )(x.reshape(blocks, _BLOCK, cin), w.reshape(cin, cout), b)
    return out.reshape(batch, height, width, cout)
```

```python
import jax
import jax.numpy as jnp
from jax import lax
import jax.experimental.pallas as pl
import jax.experimental.pallas.tpu as pltpu

_BLOCK = 4096
_STARTS = (0, 1368, 2736)
_BODY = 1344
_REST = tuple(
    end - start - _BODY for start, end in zip(_STARTS, _STARTS[1:] + (_BLOCK,))
)

_PIECE = 24
_CHUNK1 = 96
_CHUNK2 = 192
_AHEAD = 2
_RING = 4
_TAIL = 3
_WRITE_STEPS = 4
_FIRST_WRITES = 2
_REST_UNITS = 6


def _conv1x1_kernel(
    x_hbm, w_hbm, b_hbm, o_hbm, buf, w_ref, b_ref, ring, bulk, late
):
    c = buf.shape[-1]
    groups = buf.shape[0] // 4
    streams = len(_STARTS)
    steps1, steps2 = _BODY // _CHUNK1, _BODY // _CHUNK2
    n1, n2 = groups * steps1, groups * steps2
    n_rest = 2 * groups // _REST_UNITS
    n_write_steps = 2 * groups * _WRITE_STEPS
    sweeps = _CHUNK1 // _PIECE
    switch = n1 - _AHEAD + 1
    lead = _FIRST_WRITES + n_rest

    def copy(src, dst, unit, row, rows, sem, thread):
        idx = (pl.ds(2 * unit, 2), pl.ds(row, rows))
        pltpu.make_async_copy(src.at[idx], dst.at[idx], sem).start(priority=thread)

    def wait(blocks, rows, sem):
        size = buf.at[pl.ds(0, blocks), pl.ds(0, rows)]
        pltpu.make_async_copy(size, size, sem).wait()

    def read_step(i, last=False):
        g = i // steps1 if last else lax.div(i, steps1)
        j = i - g * steps1
        base = j * _CHUNK1 if last else pl.multiple_of(j * _CHUNK1, 8)
        for s in range(sweeps):
            odd_sem = late if last and s >= sweeps - _TAIL else bulk
            for start in _STARTS:
                row = base + start + s * _PIECE
                copy(x_hbm, buf, 2 * g, row, _PIECE, ring.at[i & (_RING - 1)], 0)
                copy(x_hbm, buf, 2 * g + 1, row, _PIECE, odd_sem, 1)

        def read_rest():
            for start, rows in zip(_STARTS, _REST):
                for h in range(2):
                    copy(x_hbm, buf, 2 * g + h, start + _BODY, rows, late, h)

        if last:
            read_rest()
        else:
            pl.when(j == steps1 - 1)(read_rest)

    def write_steps(lo, hi):
        rows_per_step = _BODY // _WRITE_STEPS

        def body(m, carry):
            v = lax.div(m, _WRITE_STEPS)
            r = m - v * _WRITE_STEPS
            unit = jnp.where(v < groups, 2 * v, 2 * (v - groups) + 1)
            base = pl.multiple_of(r * rows_per_step, 8)
            for s in range(rows_per_step // _PIECE):
                for start in _STARTS:
                    copy(buf, o_hbm, unit, base + start + s * _PIECE, _PIECE, bulk, 1)

            @pl.when(r == _WRITE_STEPS - 1)
            def _():
                for start, rows in zip(_STARTS, _REST):
                    copy(buf, o_hbm, unit, start + _BODY, rows, bulk, 1)

            return carry

        lax.fori_loop(lo, hi, body, 0)

    def matmul(view, starts, sizes):
        blocks = view.shape[0]
        lhs = jnp.concatenate([
            view[:, pl.ds(start, rows), :].reshape(blocks * rows, c)
            for start, rows in zip(starts, sizes)
        ])
        acc = jnp.dot(lhs, w_ref[...], preferred_element_type=jnp.float32)
        out = (acc + bias).astype(buf.dtype)
        row = 0
        for start, rows in zip(starts, sizes):
            piece = out[row:row + blocks * rows]
            view[:, pl.ds(start, rows), :] = piece.reshape(blocks, rows, c)
            row += blocks * rows

    def compute(unit, j, chunk):
        base = pl.multiple_of(j * chunk, 8)
        view = buf.at[pl.ds(2 * unit, 2), pl.ds(base, _STARTS[-1] + chunk)]
        matmul(view, _STARTS, (chunk,) * streams)

    w_copy = pltpu.make_async_copy(w_hbm, w_ref, late)
    b_copy = pltpu.make_async_copy(b_hbm, b_ref, late)

    def prologue(i, carry):
        read_step(i)

        @pl.when(i == 0)
        def _():
            w_copy.start()
            b_copy.start()

        return carry

    lax.fori_loop(0, _AHEAD, prologue, 0)
    w_copy.wait()
    b_copy.wait()
    bias = b_ref[...].astype(jnp.float32).reshape(1, c)

    def phase1(i, carry):
        @pl.when(i + _AHEAD < n1 - 1)
        def _():
            read_step(i + _AHEAD)

        @pl.when(i + _AHEAD == n1 - 1)
        def _():
            read_step(n1 - 1, last=True)

        @pl.when(i < switch)
        def _():
            wait(2, streams * _CHUNK1, ring.at[i & (_RING - 1)])

        @pl.when(i == switch)
        def _():
            tail_rows = streams * _TAIL * _PIECE
            assert tail_rows % groups == 0
            for t in range(switch, n1):
                wait(2, streams * _CHUNK1, ring.at[t % _RING])
            wait(2 * groups, streams * _BODY - tail_rows // groups, bulk)
            write_steps(0, _FIRST_WRITES)
            wait(2, tail_rows + 2 * groups * sum(_REST), late)

        g = lax.div(i, steps1)
        compute(2 * g, i - g * steps1, _CHUNK1)
        return carry

    lax.fori_loop(0, n1, phase1, 0)

    def rest(u, carry):
        view = buf.at[pl.ds(u * 2 * _REST_UNITS, 2 * _REST_UNITS)]
        matmul(view, [start + _BODY for start in _STARTS], _REST)
        write_steps(_FIRST_WRITES + u, _FIRST_WRITES + u + 1)
        return carry

    lax.fori_loop(0, n_rest, rest, 0)

    assert _FIRST_WRITES < _WRITE_STEPS and lead < 2 * _WRITE_STEPS
    for k in range(1, n2 + 1):
        g, j = divmod(k, steps2)
        assert lead + k <= (groups + g) * _WRITE_STEPS + j * _WRITE_STEPS // steps2

    def phase2(k, carry):
        g = lax.div(k, steps2)
        compute(2 * g + 1, k - g * steps2, _CHUNK2)
        write_steps(lead + k, jnp.where(k == n2 - 1, n_write_steps, lead + k + 1))
        return carry

    lax.fori_loop(0, n2, phase2, 0)
    pltpu.make_async_copy(buf, o_hbm, bulk).wait()


@jax.jit
def pallas_standalone__standard_2d_1d_3d_conv__vision_kernel(
    x: jax.Array,
    w: jax.Array,
    b: jax.Array,
):
    batch, height, width, cin = x.shape
    kh, kw, _, cout = w.shape
    blocks = batch * height * width // _BLOCK
    assert (kh, kw) == (1, 1) and cin == cout
    assert blocks * _BLOCK == batch * height * width
    assert blocks % 4 == 0 and blocks % (2 * _REST_UNITS) == 0
    hbm = pl.BlockSpec(memory_space=pltpu.HBM)
    out = pl.pallas_call(
        _conv1x1_kernel,
        in_specs=[hbm, hbm, hbm],
        out_specs=hbm,
        out_shape=jax.ShapeDtypeStruct((blocks, _BLOCK, cout), x.dtype),
        scratch_shapes=[
            pltpu.VMEM((blocks, _BLOCK, cin), x.dtype),
            pltpu.VMEM((cin, cout), w.dtype),
            pltpu.VMEM((cout,), b.dtype),
            pltpu.SemaphoreType.DMA((_RING,)),
            pltpu.SemaphoreType.DMA(()),
            pltpu.SemaphoreType.DMA(()),
        ],
        compiler_params=pltpu.CompilerParams(
            vmem_limit_bytes=120 * 2**20,
            disable_bounds_checks=True,
        ),
    )(x.reshape(blocks, _BLOCK, cin), w.reshape(cin, cout), b)
    return out.reshape(batch, height, width, cout)
```

```python
import jax
import jax.numpy as jnp
from jax import lax
import jax.experimental.pallas as pl
import jax.experimental.pallas.tpu as pltpu

_BLOCK = 4096
_STARTS = (0, 1368, 2736)
_BODY = 1344
_REST = tuple(
    end - start - _BODY for start, end in zip(_STARTS, _STARTS[1:] + (_BLOCK,))
)

_PIECE = 24
_CHUNK1 = 96
_CHUNK2 = 192
_AHEAD = 2
_LAG = 2
_RING = 4
_TAIL = 3
_WRITE_STEPS = 4
_FIRST_WRITES = 2
_REST_UNITS = 6


def _conv1x1_kernel(
    x_hbm, w_hbm, b_hbm, o_hbm, buf, w_ref, b_ref, ring, bulk, late
):
    c = buf.shape[-1]
    groups = buf.shape[0] // 4
    streams = len(_STARTS)
    steps1, steps2 = _BODY // _CHUNK1, _BODY // _CHUNK2
    n1, n2 = groups * steps1, groups * steps2
    n_rest = 2 * groups // _REST_UNITS
    n_write_steps = 2 * groups * _WRITE_STEPS
    sweeps = _CHUNK1 // _PIECE
    switch = n1 - _AHEAD + 1
    lead = _FIRST_WRITES + n_rest

    def copy(src, dst, unit, row, rows, sem, thread):
        idx = (pl.ds(2 * unit, 2), pl.ds(row, rows))
        pltpu.make_async_copy(src.at[idx], dst.at[idx], sem).start(priority=thread)

    def wait(blocks, rows, sem):
        size = buf.at[pl.ds(0, blocks), pl.ds(0, rows)]
        pltpu.make_async_copy(size, size, sem).wait()

    def read_step(i, last=False):
        g = lax.div(i, steps1)
        j = i - g * steps1
        j_odd = jnp.where(j + _LAG < steps1, j + _LAG, j + _LAG - steps1)
        even = pl.multiple_of(j * _CHUNK1, 8)
        odd = pl.multiple_of(j_odd * _CHUNK1, 8)
        for s in range(sweeps):
            odd_sem = late if last and s >= sweeps - _TAIL else bulk
            for start in _STARTS:
                row = start + s * _PIECE
                copy(x_hbm, buf, 2 * g + 1, odd + row, _PIECE, odd_sem, 1)
                copy(x_hbm, buf, 2 * g, even + row, _PIECE, ring.at[i & (_RING - 1)], 0)

        def read_rest():
            for start, rows in zip(_STARTS, _REST):
                for h in range(2):
                    copy(x_hbm, buf, 2 * g + h, start + _BODY, rows, late, h)

        if last:
            read_rest()
        else:
            pl.when(j == steps1 - 1)(read_rest)

    def write_steps(lo, hi):
        rows_per_step = _BODY // _WRITE_STEPS

        def body(m, carry):
            v = lax.div(m, _WRITE_STEPS)
            r = m - v * _WRITE_STEPS
            unit = jnp.where(v < groups, 2 * v, 2 * (v - groups) + 1)
            base = pl.multiple_of(r * rows_per_step, 8)
            for s in range(rows_per_step // _PIECE):
                for start in _STARTS:
                    copy(buf, o_hbm, unit, base + start + s * _PIECE, _PIECE, bulk, 1)

            @pl.when(r == _WRITE_STEPS - 1)
            def _():
                for start, rows in zip(_STARTS, _REST):
                    copy(buf, o_hbm, unit, start + _BODY, rows, bulk, 1)

            return carry

        lax.fori_loop(lo, hi, body, 0)

    def matmul(view, starts, sizes):
        blocks = view.shape[0]
        lhs = jnp.concatenate([
            view[:, pl.ds(start, rows), :].reshape(blocks * rows, c)
            for start, rows in zip(starts, sizes)
        ])
        acc = jnp.dot(lhs, w_ref[...], preferred_element_type=jnp.float32)
        out = (acc + bias).astype(buf.dtype)
        row = 0
        for start, rows in zip(starts, sizes):
            piece = out[row:row + blocks * rows]
            view[:, pl.ds(start, rows), :] = piece.reshape(blocks, rows, c)
            row += blocks * rows

    def compute(unit, j, chunk):
        base = pl.multiple_of(j * chunk, 8)
        view = buf.at[pl.ds(2 * unit, 2), pl.ds(base, _STARTS[-1] + chunk)]
        matmul(view, _STARTS, (chunk,) * streams)

    w_copy = pltpu.make_async_copy(w_hbm, w_ref, late)
    b_copy = pltpu.make_async_copy(b_hbm, b_ref, late)

    def prologue(i, carry):
        read_step(i)

        @pl.when(i == 0)
        def _():
            w_copy.start()
            b_copy.start()

        return carry

    lax.fori_loop(0, _AHEAD, prologue, 0)
    w_copy.wait()
    b_copy.wait()
    bias = b_ref[...].astype(jnp.float32).reshape(1, c)

    def phase1(i, carry):
        @pl.when(i + _AHEAD < n1 - 1)
        def _():
            read_step(i + _AHEAD)

        @pl.when(i + _AHEAD == n1 - 1)
        def _():
            read_step(i + _AHEAD, last=True)

        @pl.when(i < switch)
        def _():
            wait(2, streams * _CHUNK1, ring.at[i & (_RING - 1)])

        @pl.when(i == switch)
        def _():
            tail_rows = streams * _TAIL * _PIECE
            assert tail_rows % groups == 0
            for t in range(switch, n1):
                wait(2, streams * _CHUNK1, ring.at[t % _RING])
            wait(2 * groups, streams * _BODY - tail_rows // groups, bulk)
            write_steps(0, _FIRST_WRITES)
            wait(2, tail_rows + 2 * groups * sum(_REST), late)

        g = lax.div(i, steps1)
        compute(2 * g, i - g * steps1, _CHUNK1)
        return carry

    lax.fori_loop(0, n1, phase1, 0)

    def rest(u, carry):
        view = buf.at[pl.ds(u * 2 * _REST_UNITS, 2 * _REST_UNITS)]
        matmul(view, [start + _BODY for start in _STARTS], _REST)
        write_steps(_FIRST_WRITES + u, _FIRST_WRITES + u + 1)
        return carry

    lax.fori_loop(0, n_rest, rest, 0)

    assert _FIRST_WRITES < _WRITE_STEPS and lead < 2 * _WRITE_STEPS
    for k in range(1, n2 + 1):
        g, j = divmod(k, steps2)
        assert lead + k <= (groups + g) * _WRITE_STEPS + j * _WRITE_STEPS // steps2

    def phase2(k, carry):
        g = lax.div(k, steps2)
        compute(2 * g + 1, k - g * steps2, _CHUNK2)
        write_steps(lead + k, jnp.where(k == n2 - 1, n_write_steps, lead + k + 1))
        return carry

    lax.fori_loop(0, n2, phase2, 0)
    pltpu.make_async_copy(buf, o_hbm, bulk).wait()


@jax.jit
def pallas_standalone__standard_2d_1d_3d_conv__vision_kernel(
    x: jax.Array,
    w: jax.Array,
    b: jax.Array,
):
    batch, height, width, cin = x.shape
    kh, kw, _, cout = w.shape
    blocks = batch * height * width // _BLOCK
    assert (kh, kw) == (1, 1) and cin == cout
    assert blocks * _BLOCK == batch * height * width
    assert blocks % 4 == 0 and blocks % (2 * _REST_UNITS) == 0
    hbm = pl.BlockSpec(memory_space=pltpu.HBM)
    out = pl.pallas_call(
        _conv1x1_kernel,
        in_specs=[hbm, hbm, hbm],
        out_specs=hbm,
        out_shape=jax.ShapeDtypeStruct((blocks, _BLOCK, cout), x.dtype),
        scratch_shapes=[
            pltpu.VMEM((blocks, _BLOCK, cin), x.dtype),
            pltpu.VMEM((cin, cout), w.dtype),
            pltpu.VMEM((cout,), b.dtype),
            pltpu.SemaphoreType.DMA((_RING,)),
            pltpu.SemaphoreType.DMA(()),
            pltpu.SemaphoreType.DMA(()),
        ],
        compiler_params=pltpu.CompilerParams(
            vmem_limit_bytes=120 * 2**20,
            disable_bounds_checks=True,
        ),
    )(x.reshape(blocks, _BLOCK, cin), w.reshape(cin, cout), b)
    return out.reshape(batch, height, width, cout)
```
